```python
import os as _os
_os.environ.setdefault("JAX_PLATFORMS", "cpu")
import jax
import jax.numpy as jnp

def _softmax(x, axis=-1):
    return jax.nn.softmax(x, axis=axis)
def _gelu(x):
    return jax.nn.gelu(x, approximate=True)
def _silu(x):
    return jax.nn.silu(x)
def _sigmoid(x):
    return jax.nn.sigmoid(x)
def _layernorm(x, axis=-1, eps=1e-5):
    m = jnp.mean(x, axis=axis, keepdims=True)
    v = jnp.var(x, axis=axis, keepdims=True)
    return (x - m) / jnp.sqrt(v + eps)
def _scatter_add(tgt, idx, src, axis=0):
    return tgt.at[idx].add(src)
def _segment_sum(src, seg, n):
    return jax.ops.segment_sum(src, seg, n)
class _Rng:
    def __init__(self, key):
        self._k = key
    def _next(self):
        self._k, sub = jax.random.split(self._k)
        return sub
    def normal(self, shape):
        return jax.random.normal(self._next(), shape, dtype=jnp.bfloat16)
    def randint(self, lo, hi, shape):
        return jax.random.randint(self._next(), shape, lo, hi, dtype=jnp.int32)
    def uniform(self, shape, lo=0.0, hi=1.0):
        return jax.random.uniform(self._next(), shape, jnp.bfloat16, lo, hi)
    def permutation(self, n):
        return jax.random.permutation(self._next(), n)


kernel_name = 'sequential_preLN__sliding_local_dilated__dense_activation_silu__prompt'

def setup_inputs():
    _rng = _Rng(jax.random.key(int.from_bytes(__import__("os").urandom(4), "little")))
    _w = (lambda a: (lambda t: t.astype(jnp.bfloat16) if jnp.issubdtype(t.dtype, jnp.floating) else t)(jnp.asarray(a)))
    def _A_setup():
        B, S, D = 1, 2048, 1024
        return {
            "x": _w((lambda *s: _rng.normal(s) * 0.05)(B, S, D)),
            "wqkv": _w((lambda *s: _rng.normal(s) * 0.05)(D, 3 * D)),
            "wo": _w((lambda *s: _rng.normal(s) * 0.05)(D, D)),
        }
    _A_in = _A_setup()

    def _B_setup():
        B, S, D, F = 1, 2048, 1024, 3584
        return {
            "x": _w((lambda *s: _rng.normal(s) * 0.05)(B, S, D)),
            "w1": _w((lambda *s: _rng.normal(s) * 0.05)(D, F) * (D ** -0.5)),
            "w2": _w((lambda *s: _rng.normal(s) * 0.05)(F, D) * (F ** -0.5)),
        }
    _B_in = _B_setup()

    return {
        "A_x": _A_in["x"],
        "A_wqkv": _A_in["wqkv"],
        "A_wo": _A_in["wo"],
        "B_x": _B_in["x"],
        "B_w1": _B_in["w1"],
        "B_w2": _B_in["w2"],
    }

def reference(A_x, A_wqkv, A_wo, B_x, B_w1, B_w2):
    def _A_ref(x, wqkv, wo):
        B, S, D = x.shape
        H = 32; Dh = D // H
        W, dil = 8, 2
        qkv = (lambda x, *d: x.transpose(*d))((x @ wqkv).reshape(B, S, 3, H, Dh), 2, 0, 3, 1, 4)
        q, k, v = qkv[0], qkv[1], qkv[2]
        scale = Dh ** -0.5
        pos = jnp.arange(S)
        off = jnp.arange(W) * dil
        idx = pos[:, None] - off[None, :]
        mask = idx >= 0
        idx_c = jnp.where(mask, idx, 0).reshape(-1)
        kg = k[:, :, idx_c, :].reshape(B, H, S, W, Dh)
        vg = v[:, :, idx_c, :].reshape(B, H, S, W, Dh)
        logits = jnp.einsum("bhsd,bhswd->bhsw", q, kg) * scale
        logits = jnp.where(mask[None, None, :, :], logits, -1e9)
        attn = _softmax(logits, axis=-1)
        o = jnp.einsum("bhsw,bhswd->bhsd", attn, vg)
        return (lambda x, *d: x.transpose(*d))(o, 0, 2, 1, 3).reshape(B, S, D) @ wo

    def _B_ref(x, w1, w2):
        h = jnp.einsum("bsd,df->bsf", x, w1)
        h = _silu(h)
        out = jnp.einsum("bsf,fd->bsd", h, w2)
        return out

    x = A_x
    h = x + _A_ref(_layernorm(x, axis=-1), A_wqkv, A_wo)
    h2 = h + _B_ref(_layernorm(h, axis=-1), B_w1, B_w2)
    return h2
```

```python
import contextlib
import functools

import jax
import jax.numpy as jnp
from jax import lax
from jax.experimental import pallas as pl
from jax.experimental.pallas import tpu as pltpu

S, D, F = 2048, 1024, 3584
H, DH, WIN, DIL = 32, 32, 8, 2
LANE = 128
NT = D // LANE
HALO = 16
EPS = 1e-5
f32, bf16, u32 = jnp.float32, jnp.bfloat16, jnp.uint32


def _quad(X):
    h = len(X) // 2
    q = lambda i, j: [row[j * h:(j + 1) * h] for row in X[i * h:(i + 1) * h]]
    return q(0, 0), q(0, 1), q(1, 0), q(1, 1)


def _add(X, Y):
    return [[a + b for a, b in zip(r, s)] for r, s in zip(X, Y)]


def _sub(X, Y):
    return [[a - b for a, b in zip(r, s)] for r, s in zip(X, Y)]


def pre_a(A):
    if len(A) == 1:
        return [A[0][0]]
    a11, a12, a21, a22 = _quad(A)
    ops = [a11, _add(a11, a12), a22, _add(a11, a22), _sub(a12, a22), _add(a21, a22), _sub(a21, a11)]
    return [x for o in ops for x in pre_a(o)]


def pre_b(B):
    if len(B) == 1:
        return [B[0][0]]
    b11, b12, b21, b22 = _quad(B)
    ops = [_sub(b12, b22), b22, _sub(b21, b11), _add(b11, b22), _add(b21, b22), b11, _add(b11, b12)]
    return [x for o in ops for x in pre_b(o)]


def post(prod, level, base=0):
    if level == 0:
        return [[prod(base)]]
    n = 7 ** (level - 1)
    sub = lambda i: post(prod, level - 1, base + i * n)
    m3 = sub(0)
    m5 = sub(1)
    c12 = _add(m3, m5)
    m4 = sub(2)
    t = _sub(m4, m5)
    m1 = sub(3)
    t = _add(t, m1)
    u = _add(m1, m3)
    m7 = sub(4)
    c11 = _add(t, m7)
    m2 = sub(5)
    c21 = _add(m2, m4)
    u = _sub(u, m2)
    m6 = sub(6)
    c22 = _add(u, m6)
    return [r + s for r, s in zip(c11, c12)] + [r + s for r, s in zip(c21, c22)]


def _lane(rows):
    return lax.broadcasted_iota(jnp.int32, (rows, LANE), 1)


def _swap_tiles(t):
    lane = _lane(t[0].shape[0])
    t = list(t)
    for b in range(3):
        m = (lane & (4 << b)) != 0
        for j in range(NT):
            if not j & (1 << b):
                k = j | (1 << b)
                t[j], t[k] = jnp.where(m, t[k], t[j]), jnp.where(m, t[j], t[k])
    return t


def to_head_minor(t):
    lane = _lane(t[0].shape[0])
    t = _swap_tiles(t)
    head, dl = lane & 31, lane >> 5
    out = []
    for j in range(NT):
        src = ((head & 3) << 5) | (((head >> 2) ^ j) << 2) | dl
        out.append(jnp.take_along_axis(t[j], src, axis=1))
    return out


def from_head_minor(t):
    lane = _lane(t[0].shape[0])
    out = []
    for j in range(NT):
        src = ((lane & 3) << 5) | ((((lane >> 2) & 7) ^ j) << 2) | (lane >> 5)
        out.append(jnp.take_along_axis(t[j], src, axis=1))
    return _swap_tiles(out)


def pack(x):
    return pltpu.bitcast(x.astype(bf16), u32)


def unpack(w):
    return pltpu.bitcast(w, bf16)


def tiles(x):
    return [x[:, c:c + LANE] for c in range(0, x.shape[1], LANE)]


class Timeline:
    def __init__(self, never):
        self.never, self.marks, self.jobs, self.due = never, [], [], []

    def add(self, steps, chains, spans, lag=None):
        n, total, acc, at = len(steps) * chains, sum(s[2] for s in spans), 0.0, []
        for lo, hi, share in spans:
            a, acc = round(n * acc / total), acc + share
            b = round(n * acc / total)
            at += [int(lo + (hi - lo) * t / (b - a)) for t in range(b - a)]
        self.jobs += [(at[i * chains:(i + 1) * chains], step, lag) for i, step in enumerate(steps)]

    def run(self, everything=False):
        keep = []
        for at, step, lag in self.jobs:
            if at[-1] < len(self.marks) or everything:
                it = iter(at)

                def tie(x):
                    i = min(next(it), len(self.marks) - 1)
                    return x if i < 0 else jnp.where(self.never, pltpu.bitcast(self.marks[i], x.dtype), x)
                end = step(tie)
                if lag is not None:
                    self.due.append((at[-1] + lag, end))
            else:
                keep.append((at, step, lag))
        self.jobs = keep

    def dot(self, lhs, w):
        per_row = -(-w.shape[1] // (4 * LANE))
        rows = [lhs[r:r + 8] for r in range(0, lhs.shape[0], 8)]
        for g in range(len(rows)):
            now = [v for t, v in self.due if t <= len(self.marks) + 2 * g * per_row]
            self.due = [(t, v) for t, v in self.due if t > len(self.marks) + 2 * g * per_row]
            if now:
                t = tiles(rows[g])
                for q, v in enumerate(now):
                    t[q % len(t)] = jnp.where(self.never, pltpu.bitcast(v, u32), t[q % len(t)])
                rows[g] = jnp.concatenate(t, axis=1)
        y = jnp.dot(unpack(jnp.concatenate(rows, axis=0)), unpack(w), preferred_element_type=f32)
        self.marks.extend(y[r:r + 8, c:c + LANE] for r in range(0, y.shape[0], 8) for c in range(0, y.shape[1], 4 * LANE))
        self.run()
        return y


def make(TA=256, TB=256, LO=1, LF=2, NC=1, NC2=2, vmem=124, flags=None,
         w_pv=(0.0, 0.9), w_lg=(0.0, 0.9), w_ln=(0.0, 0.7), w_ln2=(0.0, 0.5), lag_lg=200,
         sh=(0.0, 0.3, 0.1, 0.6), w_cp=(0.0, 0.6), w_cl=(0.0, 0.5), scopes=False, tie_all=True, tie_ln=True, only='PAEB'):
    scope = jax.named_scope if scopes else (lambda n: contextlib.nullcontext())
    LQ = 1
    PQ, PO, PF = 2 ** LQ, 2 ** LO, 2 ** LF
    RQ, RO, RF = 7 ** LQ, 7 ** LO, 7 ** LF
    nA, nB = S // TA, S // TB
    KT = D // PQ // LANE
    NS = nA
    KI, QI, VI = 0, 1, 2
    MQ = RQ * (NT // PQ // NC) * (TA // PQ // 8)
    MO = RO * (NT // PO // NC) * (TA // PO // 8)

    def aligned(x, m):
        return x if isinstance(x, int) else pl.multiple_of(x, m)

    def layer_norm(x, scale, tie):
        t = tiles(x)
        t = [tie(a) for a in t] if tie_ln else [tie(t[0])] + t[1:]
        s = functools.reduce(lambda a, b: a + b, t)
        mean = jnp.sum(s, axis=-1, keepdims=True) * (1.0 / D)
        t = [a - mean for a in t]
        s = functools.reduce(lambda a, b: a + b, [a * a for a in t])
        var = jnp.sum(s, axis=-1, keepdims=True) * (1.0 / D)
        r = lax.rsqrt(var + EPS)
        if scale != 1.0:
            r = r * scale
        return jnp.concatenate([a * r for a in t], axis=1)

    def split_lhs(parts, dst, r):
        P = len(parts)
        kk = parts[0].shape[1] // P
        ops = pre_a([[a[:, k * kk:(k + 1) * kk] for k in range(P)] for a in parts])
        for p, o in enumerate(ops):
            dst.at[p][pl.ds(r // 2, 8), :] = pack(o)
        return ops[-1][0:8, 0:LANE]

    def norm_steps(load, T, P, dst, scale):
        m = T // P

        def step(tie, r):
            return split_lhs([jnp.concatenate([layer_norm(load(a * m + r + u), scale, tie) for u in (0, 8)], axis=0)
                              for a in range(P)], dst, r)
        return [functools.partial(step, r=r) for r in range(0, m, 16)], 2 * P * (NT if tie_ln else 1)

    def weight_steps(raw, dst, P, rows):
        kk, nn = raw.shape[0] // P, raw.shape[1] // P

        def step(tie, r):
            blocks = []
            for k in range(P):
                halves = []
                for u in (0, 8):
                    t = []
                    for c in range(0, raw.shape[1], 2 * LANE):
                        t += tiles(raw[pl.ds(aligned(k * kk + r + u, 8), 8), pl.ds(c, 2 * LANE)].astype(f32))
                    halves.append(t)
                blocks.append(halves)
            per = nn // LANE
            for c in range(per):
                for k in range(P):
                    for j in (range(P) if tie_all else [k]):
                        for u in range(2):
                            blocks[k][u][j * per + c] = tie(blocks[k][u][j * per + c])
            blocks = [[jnp.concatenate([jnp.concatenate(h[j * per:(j + 1) * per], axis=1) for h in halves], axis=0)
                       for j in range(P)] for halves in blocks]
            for p, o in enumerate(pre_b(blocks)):
                dst.at[p][pl.ds(aligned(r // 2, 8), 8), :] = pack(o)
        return [functools.partial(step, r=r) for r in rows], 2 * P * (nn // LANE) * (P if tie_all else 1)

    def kernel(x_hbm, wqkv_hbm, wo_hbm, w1_hbm, w2_hbm, o_hbm, w1t, w2t, h_buf, lhs3, flag):
        flag[0] = 0

        def block(fn):
            lax.fori_loop(flag[0], 1, lambda t, c: fn(), None)

        def timeline():
            return Timeline(flag[0] > 0)

        def alone(steps):
            tl = Timeline(None)
            tl.add(*steps, [(0, 0, 1)])
            tl.run(True)

        def matmul(tl, lhs, w, level, n, nw):
            return post(lambda p: tl.dot(lhs[p], w[p, :, pl.ds(n * nw, nw)]), level)

        def ln2(i):
            return norm_steps(lambda r: h_buf[pl.ds(aligned(i * TB + r, 8), 8), :], TB, PF, lhs3, 0.5)

        def phase_a(x_buf, wqkv_raw, wo_raw, w1_raw, w2_raw, wt, wot,
                    lhs0, lhs1, lhs2, lhs2b, qkv, p_buf, sem_x, sem_w, sem_f):
            def x_cp(i):
                rows = pl.ds(aligned(i * TA, TA), TA)
                return pltpu.make_async_copy(x_hbm.at[rows], x_buf.at[rows], sem_x.at[i])

            def w_copies(c):
                cols = pl.ds((1, 0, 2)[c // KT] * D, D)
                cps = []
                for k in range(PQ):
                    rows = pl.ds(k * (D // PQ) + c % KT * LANE, LANE)
                    cps.append(pltpu.make_async_copy(wqkv_hbm.at[rows, cols], wqkv_raw.at[rows, cols], sem_w.at[c]))
                return cps

            wo_cp = pltpu.make_async_copy(wo_hbm, wo_raw, sem_w.at[3 * KT])
            r1, r2 = D // PF // NS, F // PF // NS

            def f_cp(s):
                cps = []
                for k in range(PF):
                    a, b = aligned(k * (D // PF) + s * r1, 16), aligned(k * (F // PF) + s * r2, 16)
                    cps.append(pltpu.make_async_copy(w1_hbm.at[pl.ds(a, r1)], w1_raw.at[pl.ds(a, r1)], sem_f.at[s]))
                    cps.append(pltpu.make_async_copy(w2_hbm.at[pl.ds(b, r2)], w2_raw.at[pl.ds(b, r2)], sem_f.at[s]))
                return cps

            def start(cps):
                for cp in cps:
                    cp.start()

            def wait(cps):
                for cp in cps:
                    cp.wait()

            def prep_qkv(c):
                m, kt = divmod(c, KT)
                kk = D // PQ

                def step(tie, r):
                    blocks = []
                    for k in range(PQ):
                        w = wqkv_raw[pl.ds(k * kk + r, 16), pl.ds((1, 0, 2)[m] * D, D)]
                        t = [pltpu.bitcast(v, u32) for v in tiles(w)]
                        t = [tie(v) if j % 2 == 0 else v for j, v in enumerate(t)]
                        w = jnp.concatenate([unpack(v) for v in to_head_minor(t)], axis=1).astype(f32)
                        blocks.append([w[:, j * kk:(j + 1) * kk] for j in range(PQ)])
                    for p, o in enumerate(pre_b(blocks)):
                        wt.at[m, p][pl.ds(r // 2, 8), :] = pack(o)
                return [functools.partial(step, r=r) for r in range(kt * LANE, (kt + 1) * LANE, 16)], PQ * NT // 2

            def prep_ffn(tl, s, spans):
                tl.add(*weight_steps(w1_raw, w1t, PF, [s * r1 + r for r in range(0, r1, 16)]), spans)
                tl.add(*weight_steps(w2_raw, w2t, PF, [s * r2 + r for r in range(0, r2, 16)]), spans)

            def ln1(i, dst):
                return norm_steps(lambda r: x_buf[pl.ds(aligned(i * TA + r, 8), 8), :].astype(f32), TA, PQ, dst, 1.0)

            def logits(first, lo=0, hi=TA):
                def step(tie, r):
                    q = [tie(qkv[QI, j, pl.ds(HALO + r, 8), :]) for j in range(NT)]
                    lg = []
                    for w in range(WIN):
                        t = [q[j] * qkv[KI, j, pl.ds(HALO + r - DIL * w, 8), :] for j in range(NT)]
                        acc = functools.reduce(lambda a, b: a + b, t)
                        acc = acc + pltpu.roll(acc, 64, 1)
                        acc = acc + pltpu.roll(acc, 32, 1)
                        acc = acc * (DH ** -0.5)
                        if first and r < DIL * w:
                            pos = r + lax.broadcasted_iota(jnp.int32, (8, LANE), 0)
                            acc = jnp.where(pos >= DIL * w, acc, -1e9)
                        lg.append(acc)
                    mx = functools.reduce(jnp.maximum, lg)
                    e = [jnp.exp(t - mx) for t in lg]
                    inv = 1.0 / functools.reduce(lambda a, b: a + b, e)
                    for w in range(WIN):
                        p_buf[w, pl.ds(r, 8), :] = e[w] * inv
                    if r == TA - 8:
                        qkv[KI, :, pl.ds(0, HALO), :] = qkv[KI, :, pl.ds(TA, HALO), :]
                    return inv
                return [functools.partial(step, r=r) for r in range(lo, hi, 8)], WIN

            def values(dst):
                mo = TA // PO

                def step(tie, r):
                    parts = []
                    for a in range(PO):
                        rows = []
                        for rr in (a * mo + r, a * mo + r + 8):
                            pw = [tie(p_buf[w, pl.ds(rr, 8), :]) for w in range(WIN)]
                            o = []
                            for j in range(NT):
                                t = [pw[w] * qkv[VI, j, pl.ds(HALO + rr - DIL * w, 8), :] for w in range(WIN)]
                                o.append(functools.reduce(lambda a, b: a + b, t))
                            rows.append(jnp.concatenate(from_head_minor(o), axis=1))
                        parts.append(jnp.concatenate(rows, axis=0))
                    end = split_lhs(parts, dst, r)
                    if r == mo - 16:
                        qkv[VI, :, pl.ds(0, HALO), :] = qkv[VI, :, pl.ds(TA, HALO), :]
                    return end
                return [functools.partial(step, r=r) for r in range(0, mo, 16)], 2 * PO * NT

            def project(tl, m):
                rows, nt = TA // PQ, NT // PQ
                for n in range(nt // NC):
                    c = matmul(tl, lhs1, wt.at[m], LQ, n, NC * LANE)
                    for a in range(PQ):
                        for b in range(PQ):
                            for q, t in enumerate(tiles(c[a][b])):
                                qkv[m, b * nt + n * NC + q, pl.ds(HALO + a * rows, rows), :] = t

            def project_chunk(tl, c):
                m, kt = divmod(c, KT)
                rows, nt = TA // PQ, NT // PQ
                y = post(lambda p: tl.dot(lhs0[p, :, pl.ds(kt * LANE, LANE)],
                                          wt[m, p, pl.ds(kt * LANE // 2, LANE // 2), :]), LQ)
                for a in range(PQ):
                    for b in range(PQ):
                        for q, t in enumerate(tiles(y[a][b])):
                            at = (m, b * nt + q, pl.ds(HALO + a * rows, rows), slice(None))
                            qkv[at] = t if kt == 0 else qkv[at] + t

            def out_proj(tl, i, lhs):
                nn, mo = D // PO, TA // PO
                for n in range(nn // (NC * LANE)):
                    c = matmul(tl, lhs, wot, LO, n, NC * LANE)
                    for a in range(PO):
                        rows = pl.ds(aligned(i * TA + a * mo, 16), mo)
                        for b in range(PO):
                            cs = pl.ds(b * nn + n * NC * LANE, NC * LANE)
                            h_buf[rows, cs] = x_buf[rows, cs].astype(f32) + c[a][b]

            def span(base, size, window, share=1.0):
                return base + window[0] * size, base + window[1] * size, share

            with scope("a_start"):
                x_cp(0).start()
                start(w_copies(0))
                start(w_copies(1))
                qkv[KI, :, pl.ds(0, HALO), :] = jnp.zeros((NT, HALO, LANE), f32)
                block(lambda: x_cp(0).wait())
                alone(ln1(0, lhs0))
                block(lambda: (wait(w_copies(0)), start(w_copies(2)))[0])
                alone(prep_qkv(0))
            for c in range(3 * KT if 'P' in only else 0):
                with scope("b_chunk%02d" % c):
                    @block
                    def _():
                        if c + 1 < 3 * KT:
                            wait(w_copies(c + 1))
                        if c + 3 < 3 * KT:
                            start(w_copies(c + 3))
                        elif c + 3 == 3 * KT:
                            x_cp(1).start()
                        elif c + 2 == 3 * KT:
                            wo_cp.start()
                        else:
                            x_cp(1).wait()
                            x_cp(2).start()
                            start(f_cp(0))
                    tl = timeline()
                    if c + 1 < 3 * KT:
                        tl.add(*prep_qkv(c + 1), [span(0, MQ // KT, w_cp)])
                    else:
                        tl.add(*ln1(1, lhs1), [span(0, MQ // KT, w_cp)])
                    if c >= VI * KT:
                        q = TA // KT
                        tl.add(*logits(True, (c - VI * KT) * q, (c + 1 - VI * KT) * q), [span(0, MQ // KT, w_cl)])
                    project_chunk(tl, c)
                    tl.run(True)
            with scope("c_k1"):
                @block
                def _():
                    for j in range(NT):
                        qkv[VI, j, pl.ds(0, HALO), :] = jnp.broadcast_to(qkv[VI, j, pl.ds(HALO, 1), :], (HALO, LANE))
                tl = timeline()
                tl.add(*values(lhs2), [span(0, MQ, w_pv)])
                if 'P' in only:
                    project(tl, KI)
                    tl.run(True)
            with scope("d_q1"):
                @block
                def _():
                    wo_cp.wait()
                    x_cp(3).start()
                    start(f_cp(1))
                tl = timeline()
                tl.add(*weight_steps(wo_raw, wot, PO, range(0, D // PO, 16)), [span(0, MQ, (0.0, 0.9))])
                if 'P' in only:
                    project(tl, QI)
                    tl.run(True)

            def tile(i, _):
                @block
                def _():
                    x_cp(i + 1).wait()
                    wait(f_cp(i - 1))
                    start(f_cp(i + 1))

                    @pl.when(i + 3 < nA)
                    def _():
                        x_cp(i + 3).start()
                tl = timeline()
                tl.add(*logits(False), [span(0, MQ, w_lg)], lag_lg)
                tl.add(*ln1(i + 1, lhs1), [span(MQ, MO, w_ln)])
                tl.add(*values(lhs2), [span(MQ + MO, MQ, w_pv)])
                prep_ffn(tl, i - 1, [span(0, MQ, (0, 1), sh[0]), span(MQ, MO, (0, 1), sh[1]),
                                     span(MQ + MO, MQ, (0, 1), sh[2]), span(2 * MQ + MO, MQ, (0, 0.95), sh[3])])
                project(tl, VI)
                out_proj(tl, i - 1, lhs2)
                project(tl, KI)
                project(tl, QI)
                tl.run(True)

            with scope("i_loopA"):
                if 'A' in only:
                    lax.fori_loop(1, nA - 1, tile, None)
            with scope("j_epiA"):
                block(lambda: wait(f_cp(NS - 2) + f_cp(NS - 1)))
                tl = timeline()
                tl.add(*logits(False), [span(0, MQ, w_lg)], lag_lg)
                tl.add(*values(lhs2b), [span(MQ, MO, (0.0, 0.85))])
                prep_ffn(tl, NS - 2, [span(0, MQ, (0, 1), 0.4), span(MQ, MO, (0, 1), 0.6)])
                prep_ffn(tl, NS - 1, [span(MQ + MO, MO, (0, 0.9))])
                tl.add(*ln2(0), [span(MQ + MO, MO, (0, 0.8))])
                if 'E' in only:
                    project(tl, VI)
                    out_proj(tl, nA - 2, lhs2)
                    out_proj(tl, nA - 1, lhs2b)
                    tl.run(True)

        pl.run_scoped(
            phase_a,
            pltpu.VMEM((S, D), bf16),
            pltpu.VMEM((D, 3 * D), bf16), pltpu.VMEM((D, D), bf16),
            pltpu.VMEM((D, F), bf16), pltpu.VMEM((F, D), bf16),
            pltpu.VMEM((3, RQ, D // PQ // 2, D // PQ), u32), pltpu.VMEM((RO, D // PO // 2, D // PO), u32),
            pltpu.VMEM((RQ, TA // PQ // 2, D // PQ), u32), pltpu.VMEM((RQ, TA // PQ // 2, D // PQ), u32),
            pltpu.VMEM((RO, TA // PO // 2, D // PO), u32), pltpu.VMEM((RO, TA // PO // 2, D // PO), u32),
            pltpu.VMEM((3, NT, HALO + TA, LANE), f32), pltpu.VMEM((WIN, TA, LANE), f32),
            pltpu.SemaphoreType.DMA((nA,)), pltpu.SemaphoreType.DMA((3 * KT + 1,)), pltpu.SemaphoreType.DMA((NS,)),
        )

        def phase_b(lhs4, o_buf, sem_o):
            m = TB // PF

            def o_cp(i):
                rows = pl.ds(aligned(i * TB, TB), TB)
                return pltpu.make_async_copy(o_buf.at[rows], o_hbm.at[rows], sem_o.at[i])

            def tile(i, _):
                tl = timeline()
                n1, n2 = F // PF // (NC * LANE), D // PF // (NC2 * LANE)
                m1, m2 = RF * n1 * m // 8, RF * n2 * m // 8
                tl.add(*ln2(jnp.minimum(i + 1, nB - 1)), [(m1 + w_ln2[0] * m2, m1 + w_ln2[1] * m2, 1.0)])
                for n in range(n1):
                    c = matmul(tl, lhs3, w1t, LF, n, NC * LANE)
                    act = [[g * jnp.tanh(g) + g for g in row] for row in c]
                    for p, o in enumerate(pre_a(act)):
                        lhs4.at[p][:, pl.ds(n * NC * LANE, NC * LANE)] = pack(o)
                nn = D // PF
                for n in range(n2):
                    c = matmul(tl, lhs4, w2t, LF, n, NC2 * LANE)
                    for a in range(PF):
                        rows = pl.ds(aligned(i * TB + a * m, 16), m)
                        for b in range(PF):
                            cs = pl.ds(b * nn + n * NC2 * LANE, NC2 * LANE)
                            o_buf[rows, cs] = (h_buf[rows, cs] + c[a][b]).astype(bf16)
                tl.run(True)
                o_cp(i).start()

            with scope("l_loopB"):
                if 'B' in only:
                    lax.fori_loop(0, nB, tile, None)
            with scope("m_out"):
                for i in range(nB):
                    o_cp(i).wait()

        pl.run_scoped(
            phase_b,
            pltpu.VMEM((RF, TB // PF // 2, F // PF), u32),
            pltpu.VMEM((S, D), bf16), pltpu.SemaphoreType.DMA((nB,)),
        )

    def fn(A_x, A_wqkv, A_wo, B_x, B_w1, B_w2):
        any_spec = pl.BlockSpec(memory_space=pl.ANY)
        out = pl.pallas_call(
            kernel,
            in_specs=[any_spec] * 5,
            out_specs=any_spec,
            out_shape=jax.ShapeDtypeStruct((S, D), bf16),
            scratch_shapes=[pltpu.VMEM((RF, D // PF // 2, F // PF), u32), pltpu.VMEM((RF, F // PF // 2, D // PF), u32),
                            pltpu.VMEM((S, D), f32), pltpu.VMEM((RF, TB // PF // 2, D // PF), u32),
                            pltpu.SMEM((1,), jnp.int32)],
            compiler_params=pltpu.CompilerParams(vmem_limit_bytes=vmem * 2 ** 20, flags=flags),
        )(A_x.reshape(S, D), A_wqkv, A_wo, B_w1, B_w2)
        return out.reshape(1, S, D)

    return fn


_fn = make()


@jax.jit
def pallas_sequential_preLN__sliding_local_dilated__dense_activation_silu__prompt_kernel(
    A_x: jax.Array, A_wqkv: jax.Array, A_wo: jax.Array, B_x: jax.Array, B_w1: jax.Array, B_w2: jax.Array,
):
    return _fn(A_x, A_wqkv, A_wo, B_x, B_w1, B_w2)
```

```python
import functools
import math

import jax
import jax.numpy as jnp
from jax import lax
from jax.experimental import pallas as pl
from jax.experimental.pallas import tpu as pltpu

S, D, F = 2048, 1024, 3584
DH, WIN, DIL = 32, 8, 2
EPS = 1e-5

LANE = 128
NT = D // LANE
T = 256
TILES = S // T
HALO = 16
PA, PF = 2, 4
KH = D // PA // 2
K, Q, V, K0 = 0, 1, 2, 3
SLICES = TILES - 1
ROWS1, ROWS2 = 32, 144

f32, bf16, u32 = jnp.float32, jnp.bfloat16, jnp.uint32


def _quarters(m):
    h = len(m) // 2
    part = lambda i, j: [row[j * h:(j + 1) * h] for row in m[i * h:(i + 1) * h]]
    return part(0, 0), part(0, 1), part(1, 0), part(1, 1)


def _add(x, y):
    return [[a + b for a, b in zip(r, s)] for r, s in zip(x, y)]


def _sub(x, y):
    return [[a - b for a, b in zip(r, s)] for r, s in zip(x, y)]


def left_operands(a):
    if len(a) == 1:
        return [a[0][0]]
    a11, a12, a21, a22 = _quarters(a)
    ops = [a11, _add(a11, a12), a22, _add(a11, a22), _sub(a12, a22), _add(a21, a22), _sub(a21, a11)]
    return [x for o in ops for x in left_operands(o)]


def right_operands(b):
    if len(b) == 1:
        return [b[0][0]]
    b11, b12, b21, b22 = _quarters(b)
    ops = [_sub(b12, b22), b22, _sub(b21, b11), _add(b11, b22), _add(b21, b22), b11, _add(b11, b12)]
    return [x for o in ops for x in right_operands(o)]


def products(side):
    return 7 ** (side.bit_length() - 1)


def recombine(product, side, base=0):
    if side == 1:
        return [[product(base)]]
    nth = lambda i: recombine(product, side // 2, base + i * products(side // 2))
    m3 = nth(0)
    m5 = nth(1)
    c12 = _add(m3, m5)
    m4 = nth(2)
    t = _sub(m4, m5)
    m1 = nth(3)
    t = _add(t, m1)
    u = _add(m1, m3)
    c11 = _add(t, nth(4))
    m2 = nth(5)
    c21 = _add(m2, m4)
    u = _sub(u, m2)
    c22 = _add(u, nth(6))
    return [r + s for r, s in zip(c11, c12)] + [r + s for r, s in zip(c21, c22)]


def tiles(x):
    return [x[:, c:c + LANE] for c in range(0, x.shape[1], LANE)]


def total(xs):
    return functools.reduce(lambda a, b: a + b, xs)


def aligned(i, n):
    return i if isinstance(i, int) else pl.multiple_of(i, n)


def pack(x):
    return pltpu.bitcast(x.astype(bf16), u32)


def unpack(w):
    return pltpu.bitcast(w, bf16)


def _lane_ids(x):
    return lax.broadcasted_iota(jnp.int32, x.shape, 1)


def _swap_tiles(t):
    lane, t = _lane_ids(t[0]), list(t)
    for b in range(3):
        m = (lane & (4 << b)) != 0
        for j in range(NT):
            if not j & (1 << b):
                k = j | (1 << b)
                t[j], t[k] = jnp.where(m, t[k], t[j]), jnp.where(m, t[j], t[k])
    return t


def to_head_minor(t):
    lane = _lane_ids(t[0])
    head, dim = lane & 31, lane >> 5
    return [jnp.take_along_axis(x, ((head & 3) << 5) | (((head >> 2) ^ j) << 2) | dim, axis=1)
            for j, x in enumerate(_swap_tiles(t))]


def from_head_minor(t):
    lane = _lane_ids(t[0])
    return _swap_tiles([
        jnp.take_along_axis(x, ((lane & 3) << 5) | ((((lane >> 2) & 7) ^ j) << 2) | (lane >> 5), axis=1)
        for j, x in enumerate(t)])


class Timeline:
    def __init__(self, zero=None):
        self.zero, self.marks, self.jobs, self.due = zero, [], [], []
        self.never = None if zero is None else zero > 0

    def add(self, work, spans=((0, 0, 1),), lag=None):
        steps, ties = work
        n, weight, done, at = len(steps) * ties, sum(s[2] for s in spans), 0.0, []
        for lo, hi, share in spans:
            a, done = round(n * done / weight), done + share
            b = round(n * done / weight)
            at += [int(lo + (hi - lo) * t / (b - a)) for t in range(b - a)]
        self.jobs += [(at[i * ties:(i + 1) * ties], step, lag) for i, step in enumerate(steps)]

    def run(self, everything=True):
        waiting = []
        for at, step, lag in self.jobs:
            if not everything and at[-1] >= len(self.marks):
                waiting.append((at, step, lag))
                continue
            positions = iter(at)

            def tie(x):
                i = min(next(positions), len(self.marks) - 1)
                return x if i < 0 else jnp.where(self.never, pltpu.bitcast(self.marks[i], x.dtype), x)

            dst = step(tie)
            if lag is not None:
                self.due.append((at[-1] + lag, dst[pl.ds(aligned(self.zero * 8, 8), 8), pl.ds(0, LANE)]))
        self.jobs = waiting

    def dot(self, lhs, rhs):
        rows = [lhs[r:r + 8] for r in range(0, lhs.shape[0], 8)]
        for g in range(len(rows)):
            now = len(self.marks) + 2 * g
            ready = [v for t, v in self.due if t <= now]
            self.due = [(t, v) for t, v in self.due if t > now]
            if ready:
                t = tiles(rows[g])
                for q, v in enumerate(ready):
                    t[q % len(t)] = jnp.where(self.never, pltpu.bitcast(v, u32), t[q % len(t)])
                rows[g] = jnp.concatenate(t, axis=1)
        y = jnp.dot(unpack(jnp.concatenate(rows, axis=0)), unpack(rhs), preferred_element_type=f32)
        self.marks.extend(y[r:r + 8, 0:LANE] for r in range(0, y.shape[0], 8))
        self.run(everything=False)
        return y


def alone(work):
    line = Timeline()
    line.add(work)
    line.run()


def span(base, size, lo, hi, share=1.0):
    return base + lo * size, base + hi * size, share


def store_left(parts, dst, r):
    side = len(parts)
    width = parts[0].shape[1] // side
    for p, o in enumerate(left_operands([[a[:, k * width:(k + 1) * width] for k in range(side)] for a in parts])):
        dst.at[p][pl.ds(r // 2, 8), :] = pack(o)
    return dst.at[0]


def layer_norm(load, side, dst, scale, tie_all):
    m, per = T // side, NT // side

    def stats(x, tie):
        t = tiles(x)
        t = [tie(a) for a in t] if tie_all else [tie(t[0])] + t[1:]
        mean = jnp.sum(total(t), axis=-1, keepdims=True) * (1.0 / D)
        t = [a - mean for a in t]
        var = jnp.sum(total([a * a for a in t]), axis=-1, keepdims=True) * (1.0 / D)
        r = lax.rsqrt(var + EPS)
        return mean, r if scale == 1.0 else r * scale

    def step(tie, r):
        rows = [a * m + r + u for a in range(side) for u in (0, 8)]
        moments = [stats(load(q), tie) for q in rows]
        t = [tiles(load(q)) for q in rows]
        for c in range(per):
            for k in range(side):
                for g, (mean, _) in enumerate(moments):
                    t[g][k * per + c] = tie(t[g][k * per + c]) - mean
        y = [jnp.concatenate([v * s for v in row], axis=1) for row, (_, s) in zip(t, moments)]
        return store_left([jnp.concatenate(y[2 * a:2 * a + 2], axis=0) for a in range(side)], dst, r)

    return ([functools.partial(step, r=r) for r in range(0, m, 16)],
            2 * side * ((NT if tie_all else 1) + NT))


def weights(raw, dst, rows, woven=False):
    side, width = raw.shape[0], raw.shape[2]
    per = width // LANE // side

    def step(tie, r):
        t = [[[v for c in range(0, width, 2 * LANE)
               for v in tiles(raw.at[k][pl.ds(aligned(r + u, 8), 8), pl.ds(c, 2 * LANE)].astype(f32))]
              for u in (0, 8)] for k in range(side)]
        if woven:
            t = [[[h[c * side + j] for j in range(side) for c in range(per)] for h in halves] for halves in t]
        for c in range(per):
            for k in range(side):
                for j in range(side):
                    for h in t[k]:
                        h[j * per + c] = tie(h[j * per + c])
        blocks = [[jnp.concatenate([jnp.concatenate(h[j * per:(j + 1) * per], axis=1) for h in halves], axis=0)
                   for j in range(side)] for halves in t]
        for p, o in enumerate(right_operands(blocks)):
            dst.at[p][pl.ds(aligned(r // 2, 8), 8), :] = pack(o)
        return dst.at[0]

    return [functools.partial(step, r=r) for r in rows], 2 * side * side * per


def kernel(x_hbm, wqkv_hbm, wo_hbm, w1_hbm, w2_hbm, out_hbm, w1, w2, h_buf, hn, zero):
    zero[0] = 0

    def apart(fn):
        lax.fori_loop(zero[0], 1, lambda i, carry: fn(), None)

    def timeline():
        return Timeline(zero[0])

    def norm_h(i):
        return layer_norm(lambda r: h_buf[pl.ds(aligned(i * T + r, 8), 8), :], PF, hn, 0.5, False)

    def attention(x_buf, wqkv_raw, wo_raw, w1_raw, w2_raw, wqkv0, wqkv1, wo,
                  xn_first, xn, att, att_last, qkv, probs, x_sem, w_sem, f_sem):
        wqkv = (wqkv0, wqkv1)
        rows, nt = T // PA, NT // PA
        whole = products(PA) * nt * (rows // 8)

        def columns(m):
            return aligned((1 - m + 3 * (m >> 1)) * D, D)

        def x_copy(i):
            at = pl.ds(aligned(i * T, T), T)
            return pltpu.make_async_copy(x_hbm.at[at], x_buf.at[at], x_sem.at[i])

        def wqkv_copy(m, half):
            at = (slice(None), pl.ds(half * KH, KH), pl.ds(columns(m), D))
            return pltpu.make_async_copy(wqkv_hbm.at[at], wqkv_raw.at[at], w_sem.at[2 * m + half])

        def wo_copy():
            return pltpu.make_async_copy(wo_hbm, wo_raw, w_sem.at[6])

        def slice_rows(last):
            return (D // PF - (SLICES - 1) * ROWS1, F // PF - (SLICES - 1) * ROWS2) if last else (ROWS1, ROWS2)

        def slice_copies(s, last=False):
            n1, n2 = slice_rows(last)
            a, b = pl.ds(aligned(s * ROWS1, 16), n1), pl.ds(aligned(s * ROWS2, 16), n2)
            return [pltpu.make_async_copy(w1_hbm.at[:, a], w1_raw.at[:, a], f_sem.at[2 * s]),
                    pltpu.make_async_copy(w2_hbm.at[:, b], w2_raw.at[:, b], f_sem.at[2 * s + 1])]

        def start(copies):
            for c in copies:
                c.start()

        def wait(copies):
            for c in copies:
                c.wait()

        def projection_weights(m, half, group):
            col0, width = columns(m), D // PA

            def step(tie, r):
                t = []
                for j in range(NT):
                    pieces = []
                    for k in range(PA):
                        at = (pl.ds(half * KH + r, group), pl.ds(aligned(col0 + j * LANE, LANE), LANE))
                        w = pltpu.bitcast(wqkv_raw.at[k][at], u32)
                        pieces += [tie(w[u:u + 8]) if j % 2 == 0 else w[u:u + 8] for u in range(0, group // 2, 8)]
                    t.append(jnp.concatenate(pieces, axis=0))
                w = jnp.concatenate([unpack(v) for v in to_head_minor(t)], axis=1).astype(f32)
                blocks = [[w[k * group:(k + 1) * group, j * width:(j + 1) * width] for j in range(PA)]
                          for k in range(PA)]
                for p, o in enumerate(right_operands(blocks)):
                    wqkv[half].at[m, p][pl.ds(r // 2, group // 2), :] = pack(o)
                return wqkv[half].at[0, 0]

            return [functools.partial(step, r=r) for r in range(0, KH, group)], group // 16 * PA * NT // 2

        def feed_forward_weights(line, s, last, spans, lag):
            n1, n2 = slice_rows(last)
            line.add(weights(w1_raw, w1, [s * ROWS1 + r for r in range(0, n1, 16)]), spans, lag)
            line.add(weights(w2_raw, w2, [s * ROWS2 + r for r in range(0, n2, 16)], woven=True), spans, lag)

        def norm_x(i, dst, tie_all=True):
            return layer_norm(lambda r: x_buf[pl.ds(aligned(i * T + r, 8), 8), :].astype(f32), PA, dst, 1.0, tie_all)

        def scores(first):
            keys = K0 if first else K

            def step(tie, r):
                q = [tie(qkv[Q, j, pl.ds(HALO + r, 8), :]) for j in range(NT)]
                logits = []
                for w in range(WIN):
                    s = total([q[j] * qkv[keys, j, pl.ds(HALO + r - DIL * w, 8), :] for j in range(NT)])
                    s = s + pltpu.roll(s, 64, 1)
                    s = s + pltpu.roll(s, 32, 1)
                    if first and r < DIL * w:
                        pos = r + lax.broadcasted_iota(jnp.int32, s.shape, 0)
                        s = jnp.where(pos >= DIL * w, s, -1e9 * DH ** 0.5)
                    logits.append(s)
                top = functools.reduce(jnp.maximum, logits)
                e = [jnp.exp2((s - top) * (DH ** -0.5 * math.log2(math.e))) for s in logits]
                inv = 1.0 / total(e)
                for w in range(WIN):
                    probs[w, pl.ds(r, 8), :] = e[w] * inv
                if r == T - 8:
                    qkv[K, :, pl.ds(0, HALO), :] = qkv[keys, :, pl.ds(T, HALO), :]
                return probs.at[0]

            return [functools.partial(step, r=r) for r in range(0, T, 8)], WIN

        def mix_values(dst):
            def step(tie, r):
                mixed = []
                for a in range(PA):
                    o = [[] for _ in range(NT)]
                    for q in (a * rows + r, a * rows + r + 8):
                        p = [tie(probs[w, pl.ds(q, 8), :]) for w in range(WIN)]
                        for j in range(NT):
                            o[j].append(total([p[w] * qkv[V, j, pl.ds(HALO + q - DIL * w, 8), :] for w in range(WIN)]))
                    mixed.append(o)
                parts = [jnp.concatenate(from_head_minor([jnp.concatenate(c, axis=0) for c in o]), axis=1)
                         for o in mixed]
                written = store_left(parts, dst, r)
                if r == rows - 16:
                    qkv[V, :, pl.ds(0, HALO), :] = qkv[V, :, pl.ds(T, HALO), :]
                return written

            return [functools.partial(step, r=r) for r in range(0, rows, 16)], 2 * PA * WIN

        def project(line, m):
            for n in range(nt):
                cols = pl.ds(n * LANE, LANE)
                c = recombine(lambda p: line.dot(xn[p], jnp.concatenate([w[m, p, :, cols] for w in wqkv], axis=0)), PA)
                for a in range(PA):
                    for b in range(PA):
                        qkv[m, b * nt + n, pl.ds(HALO + a * rows, rows), :] = c[a][b]

        def project_first(line, m, half):
            slot = m if isinstance(m, int) else jnp.where(m == K, K0, m)
            for n in range(0, nt, 2):
                c = recombine(lambda p: line.dot(xn_first[p, :, pl.ds(half * KH, KH)],
                                                 wqkv[half][m, p, :, pl.ds(n * LANE, 2 * LANE)]), PA)
                for a in range(PA):
                    for b in range(PA):
                        for q, t in enumerate(tiles(c[a][b])):
                            at = (slot, b * nt + n + q, pl.ds(HALO + a * rows, rows), slice(None))
                            qkv[at] = t if half == 0 else qkv[at] + t

        def project_out(line, i, lhs):
            for n in range(nt):
                c = recombine(lambda p: line.dot(lhs[p], wo[p, :, pl.ds(n * LANE, LANE)]), PA)
                for a in range(PA):
                    at = pl.ds(aligned(i * T + a * rows, 16), rows)
                    for b in range(PA):
                        cols = pl.ds((b * nt + n) * LANE, LANE)
                        h_buf[at, cols] = x_buf[at, cols].astype(f32) + c[a][b]

        x_copy(0).start()
        wqkv_copy(K, 0).start()
        qkv[K0, :, pl.ds(0, HALO), :] = jnp.zeros((NT, HALO, LANE), f32)

        @apart
        def _():
            x_copy(0).wait()
            wqkv_copy(K, 1).start()
        alone(norm_x(0, xn_first))

        @apart
        def _():
            wqkv_copy(K, 0).wait()
            wqkv_copy(Q, 0).start()
        alone(projection_weights(K, 0, 64))

        def first_tile(m, _):
            after = jnp.minimum(m + 1, V)

            @apart
            def _():
                wqkv_copy(m, 1).wait()
                pl.when(m < V)(lambda: wqkv_copy(after, 1).start())
                pl.when(m == V)(lambda: x_copy(1).start())
            line = timeline()
            line.add(projection_weights(m, 1, 16), [span(0, whole // 2, 0.0, 0.85)])
            project_first(line, m, 0)
            line.run()

            @pl.when(m < V)
            def _():
                @apart
                def _():
                    wqkv_copy(after, 0).wait()
                    pl.when(m == K)(lambda: wqkv_copy(V, 0).start())
                line = timeline()
                line.add(projection_weights(after, 0, 16), [span(0, whole // 2, 0.0, 0.85)])
                project_first(line, m, 1)
                line.run()

        lax.fori_loop(0, 3, first_tile, None)

        @apart
        def _():
            wo_copy().start()
            x_copy(1).wait()
        line = timeline()
        line.add(norm_x(1, xn, tie_all=False), [span(0, whole // 2, 0.0, 0.9)], 40)
        project_first(line, V, 1)
        line.run()

        apart(lambda: start([x_copy(2)] + slice_copies(0)))
        line = timeline()
        for j in range(NT):
            qkv[V, j, pl.ds(0, HALO), :] = jnp.broadcast_to(qkv[V, j, pl.ds(HALO, 1), :], (HALO, LANE))
        line.add(scores(first=True), [span(0, whole, 0.02, 0.87)])
        project(line, K)
        line.run()

        @apart
        def _():
            wo_copy().wait()
            x_copy(3).start()
        line = timeline()
        line.add(mix_values(att), [span(0, whole, 0.0, 0.95)])
        line.add(weights(wo_raw, wo, range(0, D // PA, 16)), [span(0, whole, 0.0, 0.98)])
        project(line, Q)
        line.run()
        apart(lambda: start(slice_copies(1)))

        def tile(i, _):
            x_copy(i + 1).wait()
            wait(slice_copies(i - 1))

            @pl.when(i + 3 < TILES)
            def _():
                x_copy(i + 3).start()
                start(slice_copies(i + 1))

            @pl.when(i + 3 == TILES)
            def _():
                start(slice_copies(SLICES - 1, last=True))

            line = timeline()
            line.add(scores(first=False), [span(0, whole, 0.02, 1.15)], 200)
            line.add(norm_x(i + 1, xn), [span(whole, whole, 0.2, 0.8)], 150)
            line.add(mix_values(att), [span(2 * whole, whole, 0.0, 0.95)], 150)
            feed_forward_weights(line, i - 1, False,
                                 [span(0, whole, 0, 1, 0.05), span(whole, whole, 0, 1, 0.1),
                                  span(2 * whole, whole, 0, 1, 0.15), span(3 * whole, whole, 0, 0.95, 0.7)], 250)
            project(line, V)
            project_out(line, i - 1, att)
            project(line, K)
            project(line, Q)
            line.run()

        lax.fori_loop(1, TILES - 1, tile, None)

        wait(slice_copies(SLICES - 1, last=True))
        line = timeline()
        line.add(scores(first=False), [span(0, whole, 0.0, 0.9)], 300)
        line.add(mix_values(att_last), [span(whole, whole, 0.0, 0.85)], 250)
        feed_forward_weights(line, SLICES - 1, True,
                             [span(0, whole, 0, 1, 0.2), span(2 * whole, whole, 0, 0.9, 0.8)], 250)
        line.add(norm_h(0), [span(2 * whole, whole, -0.6, 0.8)], 100)
        project(line, V)
        project_out(line, TILES - 2, att)
        project_out(line, TILES - 1, att_last)
        line.run()

    left = pltpu.VMEM((products(PA), T // PA // 2, D // PA), u32)
    half = pltpu.VMEM((3, products(PA), KH // 2, D // PA), u32)
    pl.run_scoped(
        attention,
        pltpu.VMEM((S, D), bf16),
        pltpu.VMEM((PA, D // PA, 3 * D), bf16), pltpu.VMEM((PA, D // PA, D), bf16),
        pltpu.VMEM((PF, D // PF, F), bf16), pltpu.VMEM((PF, F // PF, D), bf16),
        half, half, pltpu.VMEM((products(PA), D // PA // 2, D // PA), u32),
        left, left, left, left,
        pltpu.VMEM((4, NT, HALO + T, LANE), f32), pltpu.VMEM((WIN, T, LANE), f32),
        pltpu.SemaphoreType.DMA((TILES,)), pltpu.SemaphoreType.DMA((7,)), pltpu.SemaphoreType.DMA((2 * SLICES,)),
    )

    def feed_forward(act, out_buf, out_sem):
        rows, n1, n2 = T // PF, F // PF // LANE, D // PF // LANE
        each = products(PF) * (rows // 8)

        def out_copy(i, piece):
            r, n, c = ((0, T, 0), (0, T // 2, D // 2), (T // 2, T // 2, D // 2))[piece]
            at = (pl.ds(aligned(i * T + r, 16), n), pl.ds(c, D // 2))
            return pltpu.make_async_copy(out_buf.at[at], out_hbm.at[at], out_sem.at[3 * i + piece])

        def tile(i, _):
            line = timeline()
            line.add(norm_h(jnp.minimum(i + 1, TILES - 1)),
                     [span(n1 * each, n2 * each, 0.05, 0.4), span(n1 * each, n2 * each, 0.52, 0.88)], 60)
            for n in range(n1):
                c = recombine(lambda p: line.dot(hn[p], w1[p, :, pl.ds(n * LANE, LANE)]), PF)

                def step(tie, r, n=n, c=c):
                    g = [[jnp.concatenate([tie(b[r:r + 8]), tie(b[r + 8:r + 16])], axis=0) for b in row] for row in c]
                    for p, o in enumerate(left_operands([[b * jnp.tanh(b) + b for b in row] for row in g])):
                        act.at[p][pl.ds(r // 2, 8), pl.ds(n * LANE, LANE)] = pack(o)
                    return act.at[0]

                silu = [functools.partial(step, r=r) for r in range(0, rows, 16)], 2 * PF * PF
                if n < n1 - 1:
                    line.add(silu, [span((n + 1) * each, each, -0.15, 0.45)])
                else:
                    alone(silu)
            for n in range(n2):
                c = recombine(lambda p: line.dot(act[p], w2[p, :, pl.ds(n * LANE, LANE)]), PF)
                for a in range(PF):
                    at = (pl.ds(aligned(i * T + a * rows, 16), rows), pl.ds(n * PF * LANE, PF * LANE))
                    out_buf[at] = (h_buf[at] + jnp.concatenate(c[a], axis=1)).astype(bf16)
                    if n == 1 and a == PF // 2 - 1:
                        out_copy(i, 1).start()
                if n == 0:
                    out_copy(i, 0).start()
            line.run()
            out_copy(i, 2).start()

        lax.fori_loop(0, TILES, tile, None)
        for i in range(TILES):
            for piece in range(3):
                out_copy(i, piece).wait()

    pl.run_scoped(
        feed_forward,
        pltpu.VMEM((products(PF), T // PF // 2, F // PF), u32),
        pltpu.VMEM((S, D), bf16), pltpu.SemaphoreType.DMA((3 * TILES,)),
    )


@jax.jit
def pallas_sequential_preLN__sliding_local_dilated__dense_activation_silu__prompt_kernel(
    A_x: jax.Array,
    A_wqkv: jax.Array,
    A_wo: jax.Array,
    B_x: jax.Array,
    B_w1: jax.Array,
    B_w2: jax.Array,
):
    del B_x
    hbm = pl.BlockSpec(memory_space=pl.ANY)
    out = pl.pallas_call(
        kernel,
        in_specs=[hbm] * 5,
        out_specs=hbm,
        out_shape=jax.ShapeDtypeStruct((S, D), bf16),
        scratch_shapes=[
            pltpu.VMEM((products(PF), D // PF // 2, F // PF), u32),
            pltpu.VMEM((products(PF), F // PF // 2, D // PF), u32),
            pltpu.VMEM((S, D), f32),
            pltpu.VMEM((products(PF), T // PF // 2, D // PF), u32),
            pltpu.SMEM((1,), jnp.int32),
        ],
        compiler_params=pltpu.CompilerParams(vmem_limit_bytes=124 * 2 ** 20),
    )(A_x.reshape(S, D), A_wqkv.reshape(PA, D // PA, 3 * D), A_wo.reshape(PA, D // PA, D),
      B_w1.reshape(PF, D // PF, F), B_w2.reshape(PF, F // PF, D))
    return out.reshape(1, S, D)
```

```python
import functools
import math

import jax
import jax.numpy as jnp
from jax import lax
from jax.experimental import pallas as pl
from jax.experimental.pallas import tpu as pltpu

S, D, F = 2048, 1024, 3584
DH, WIN, DIL = 32, 8, 2
EPS = 1e-5

LANE = 128
NT = D // LANE
T = 256
TILES = S // T
HALO = 16
PA, PF = 2, 4
KH = D // PA // 2
K, Q, V, K0 = 0, 1, 2, 3
SLICES = TILES - 1
ROWS1, ROWS2 = 32, 144

f32, bf16, u32 = jnp.float32, jnp.bfloat16, jnp.uint32


def _quarters(m):
    h = len(m) // 2
    part = lambda i, j: [row[j * h:(j + 1) * h] for row in m[i * h:(i + 1) * h]]
    return part(0, 0), part(0, 1), part(1, 0), part(1, 1)


def _add(x, y):
    return [[a + b for a, b in zip(r, s)] for r, s in zip(x, y)]


def _sub(x, y):
    return [[a - b for a, b in zip(r, s)] for r, s in zip(x, y)]


def left_operands(a):
    if len(a) == 1:
        return [a[0][0]]
    a11, a12, a21, a22 = _quarters(a)
    ops = [a11, _add(a11, a12), a22, _add(a11, a22), _sub(a12, a22), _add(a21, a22), _sub(a21, a11)]
    return [x for o in ops for x in left_operands(o)]


def right_operands(b):
    if len(b) == 1:
        return [b[0][0]]
    b11, b12, b21, b22 = _quarters(b)
    ops = [_sub(b12, b22), b22, _sub(b21, b11), _add(b11, b22), _add(b21, b22), b11, _add(b11, b12)]
    return [x for o in ops for x in right_operands(o)]


def products(side):
    return 7 ** (side.bit_length() - 1)


def recombine(product, side, base=0):
    if side == 1:
        return [[product(base)]]
    nth = lambda i: recombine(product, side // 2, base + i * products(side // 2))
    m3 = nth(0)
    m5 = nth(1)
    c12 = _add(m3, m5)
    m4 = nth(2)
    t = _sub(m4, m5)
    m1 = nth(3)
    t = _add(t, m1)
    u = _add(m1, m3)
    c11 = _add(t, nth(4))
    m2 = nth(5)
    c21 = _add(m2, m4)
    u = _sub(u, m2)
    c22 = _add(u, nth(6))
    return [r + s for r, s in zip(c11, c12)] + [r + s for r, s in zip(c21, c22)]


def tiles(x):
    return [x[:, c:c + LANE] for c in range(0, x.shape[1], LANE)]


def total(xs):
    return functools.reduce(lambda a, b: a + b, xs)


def aligned(i, n):
    return i if isinstance(i, int) else pl.multiple_of(i, n)


def pack(x):
    return pltpu.bitcast(x.astype(bf16), u32)


def unpack(w):
    return pltpu.bitcast(w, bf16)


def _lane_ids(x):
    return lax.broadcasted_iota(jnp.int32, x.shape, 1)


def _swap_tiles(t):
    lane, t = _lane_ids(t[0]), list(t)
    for b in range(3):
        m = (lane & (4 << b)) != 0
        for j in range(NT):
            if not j & (1 << b):
                k = j | (1 << b)
                t[j], t[k] = jnp.where(m, t[k], t[j]), jnp.where(m, t[j], t[k])
    return t


def to_head_minor(t):
    lane = _lane_ids(t[0])
    head, dim = lane & 31, lane >> 5
    return [jnp.take_along_axis(x, ((head & 3) << 5) | (((head >> 2) ^ j) << 2) | dim, axis=1)
            for j, x in enumerate(_swap_tiles(t))]


def from_head_minor(t):
    lane = _lane_ids(t[0])
    return _swap_tiles([
        jnp.take_along_axis(x, ((lane & 3) << 5) | ((((lane >> 2) & 7) ^ j) << 2) | (lane >> 5), axis=1)
        for j, x in enumerate(t)])


class Timeline:
    def __init__(self, zero=None):
        self.zero, self.marks, self.jobs, self.due = zero, [], [], []
        self.never = None if zero is None else zero > 0

    def add(self, work, spans=((0, 0, 1),), lag=None):
        steps, ties = work
        n, weight, done, at = len(steps) * ties, sum(s[2] for s in spans), 0.0, []
        for lo, hi, share in spans:
            a, done = round(n * done / weight), done + share
            b = round(n * done / weight)
            at += [int(lo + (hi - lo) * t / (b - a)) for t in range(b - a)]
        self.jobs += [(at[i * ties:(i + 1) * ties], step, lag) for i, step in enumerate(steps)]

    def run(self, everything=True):
        waiting = []
        for at, step, lag in self.jobs:
            if not everything and at[-1] >= len(self.marks):
                waiting.append((at, step, lag))
                continue
            positions = iter(at)

            def tie(x):
                i = min(next(positions), len(self.marks) - 1)
                return x if i < 0 else jnp.where(self.never, pltpu.bitcast(self.marks[i], x.dtype), x)

            dst = step(tie)
            if lag is not None:
                self.due.append((at[-1] + lag, dst[pl.ds(aligned(self.zero * 8, 8), 8), pl.ds(0, LANE)]))
        self.jobs = waiting

    def dot(self, lhs, rhs):
        rows = [lhs[r:r + 8] for r in range(0, lhs.shape[0], 8)]
        for g in range(len(rows)):
            now = len(self.marks) + 2 * g
            ready = [v for t, v in self.due if t <= now]
            self.due = [(t, v) for t, v in self.due if t > now]
            if ready:
                t = tiles(rows[g])
                for q, v in enumerate(ready):
                    t[q % len(t)] = jnp.where(self.never, pltpu.bitcast(v, u32), t[q % len(t)])
                rows[g] = jnp.concatenate(t, axis=1)
        y = jnp.dot(unpack(jnp.concatenate(rows, axis=0)), unpack(rhs), preferred_element_type=f32)
        self.marks.extend(y[r:r + 8, 0:LANE] for r in range(0, y.shape[0], 8))
        self.run(everything=False)
        return y


def alone(work):
    line = Timeline()
    line.add(work)
    line.run()


def span(base, size, lo, hi, share=1.0):
    return base + lo * size, base + hi * size, share


def store_left(parts, dst, r):
    side = len(parts)
    width = parts[0].shape[1] // side
    for p, o in enumerate(left_operands([[a[:, k * width:(k + 1) * width] for k in range(side)] for a in parts])):
        dst.at[p][pl.ds(r // 2, 8), :] = pack(o)
    return dst.at[0]


def layer_norm(load, side, dst, scale, tie_all):
    m, per = T // side, NT // side

    def stats(x, tie):
        t = tiles(x)
        t = [tie(a) for a in t] if tie_all else [tie(t[0])] + t[1:]
        mean = jnp.sum(total(t), axis=-1, keepdims=True) * (1.0 / D)
        t = [a - mean for a in t]
        var = jnp.sum(total([a * a for a in t]), axis=-1, keepdims=True) * (1.0 / D)
        r = lax.rsqrt(var + EPS)
        return mean, r if scale == 1.0 else r * scale

    def step(tie, r):
        rows = [a * m + r + u for a in range(side) for u in (0, 8)]
        moments = [stats(load(q), tie) for q in rows]
        t = [tiles(load(q)) for q in rows]
        for c in range(per):
            for k in range(side):
                for g, (mean, _) in enumerate(moments):
                    t[g][k * per + c] = tie(t[g][k * per + c]) - mean
        y = [jnp.concatenate([v * s for v in row], axis=1) for row, (_, s) in zip(t, moments)]
        return store_left([jnp.concatenate(y[2 * a:2 * a + 2], axis=0) for a in range(side)], dst, r)

    return ([functools.partial(step, r=r) for r in range(0, m, 16)],
            2 * side * ((NT if tie_all else 1) + NT))


def weights(raw, dst, groups, woven=False):
    side, width = raw.shape[0], raw.shape[2]
    per = width // LANE // side

    def step(tie, g):
        src = [pl.ds(aligned(16 * g, 8), 8), pl.ds(aligned(16 * g + 8, 8), 8)]
        t = [[[v for c in range(0, width, 2 * LANE) for v in tiles(raw.at[k][at, pl.ds(c, 2 * LANE)].astype(f32))]
              for at in src] for k in range(side)]
        if woven:
            t = [[[h[c * side + j] for j in range(side) for c in range(per)] for h in halves] for halves in t]
        for c in range(per):
            for k in range(side):
                for j in range(side):
                    for h in t[k]:
                        h[j * per + c] = tie(h[j * per + c])
        blocks = [[jnp.concatenate([jnp.concatenate(h[j * per:(j + 1) * per], axis=1) for h in halves], axis=0)
                   for j in range(side)] for halves in t]
        at = pl.ds(aligned(8 * g, 8), 8)
        for p, o in enumerate(right_operands(blocks)):
            dst.at[p][at, :] = pack(o)
        return dst.at[0]

    return [functools.partial(step, g=g) for g in groups], 2 * side * side * per


def kernel(x_hbm, wqkv_hbm, wo_hbm, w1_hbm, w2_hbm, out_hbm, w1, w2, h_buf, hn, zero):
    zero[0] = 0

    def apart(fn):
        lax.fori_loop(zero[0], 1, lambda i, carry: fn(), None)

    def timeline():
        return Timeline(zero[0])

    def norm_h(i):
        return layer_norm(lambda r: h_buf[pl.ds(aligned(i * T + r, 8), 8), :], PF, hn, 0.5, False)

    def attention(x_buf, wqkv_raw, wo_raw, w1_raw, w2_raw, wqkv0, wqkv1, wo,
                  xn_first, xn, att, att_last, qkv, probs, x_sem, w_sem, f_sem):
        wqkv = (wqkv0, wqkv1)
        rows, nt = T // PA, NT // PA
        whole = products(PA) * nt * (rows // 8)

        def columns(m):
            return aligned((1 - m + 3 * (m >> 1)) * D, D)

        def x_copy(i):
            at = pl.ds(aligned(i * T, T), T)
            return pltpu.make_async_copy(x_hbm.at[at], x_buf.at[at], x_sem.at[i])

        def wqkv_copy(m, half):
            at = (slice(None), pl.ds(half * KH, KH), pl.ds(columns(m), D))
            return pltpu.make_async_copy(wqkv_hbm.at[at], wqkv_raw.at[at], w_sem.at[2 * m + half])

        def wo_copy():
            return pltpu.make_async_copy(wo_hbm, wo_raw, w_sem.at[6])

        def slice_rows(last):
            return (D // PF - (SLICES - 1) * ROWS1, F // PF - (SLICES - 1) * ROWS2) if last else (ROWS1, ROWS2)

        def slice_copies(s, last=False):
            n1, n2 = slice_rows(last)
            a, b = pl.ds(aligned(s * ROWS1, 16), n1), pl.ds(aligned(s * ROWS2, 16), n2)
            return [pltpu.make_async_copy(w1_hbm.at[:, a], w1_raw.at[:, a], f_sem.at[2 * s]),
                    pltpu.make_async_copy(w2_hbm.at[:, b], w2_raw.at[:, b], f_sem.at[2 * s + 1])]

        def start(copies):
            for c in copies:
                c.start()

        def wait(copies):
            for c in copies:
                c.wait()

        def projection_weights(m, half, group):
            col0, width = columns(m), D // PA
            cols = [pl.ds(aligned(col0 + j * LANE, LANE), LANE) for j in range(NT)]

            def step(tie, r):
                t = []
                for j in range(NT):
                    pieces = []
                    for k in range(PA):
                        w = pltpu.bitcast(wqkv_raw.at[k][pl.ds(half * KH + r, group), cols[j]], u32)
                        pieces += [tie(w[u:u + 8]) if j % 2 == 0 else w[u:u + 8] for u in range(0, group // 2, 8)]
                    t.append(jnp.concatenate(pieces, axis=0))
                w = jnp.concatenate([unpack(v) for v in to_head_minor(t)], axis=1).astype(f32)
                blocks = [[w[k * group:(k + 1) * group, j * width:(j + 1) * width] for j in range(PA)]
                          for k in range(PA)]
                for p, o in enumerate(right_operands(blocks)):
                    wqkv[half].at[m, p][pl.ds(r // 2, group // 2), :] = pack(o)
                return wqkv[half].at[0, 0]

            return [functools.partial(step, r=r) for r in range(0, KH, group)], group // 16 * PA * NT // 2

        def feed_forward_weights(line, s, last, spans, lag):
            n1, n2 = slice_rows(last)
            line.add(weights(w1_raw, w1, [s * (ROWS1 // 16) + g for g in range(n1 // 16)]), spans, lag)
            line.add(weights(w2_raw, w2, [s * (ROWS2 // 16) + g for g in range(n2 // 16)], woven=True), spans, lag)

        def norm_x(i, dst, tie_all=True):
            return layer_norm(lambda r: x_buf[pl.ds(aligned(i * T + r, 8), 8), :].astype(f32), PA, dst, 1.0, tie_all)

        def scores(first):
            keys = K0 if first else K

            def step(tie, r):
                q = [tie(qkv[Q, j, pl.ds(HALO + r, 8), :]) for j in range(NT)]
                logits = []
                for w in range(WIN):
                    s = total([q[j] * qkv[keys, j, pl.ds(HALO + r - DIL * w, 8), :] for j in range(NT)])
                    s = s + pltpu.roll(s, 64, 1)
                    s = s + pltpu.roll(s, 32, 1)
                    if first and r < DIL * w:
                        pos = r + lax.broadcasted_iota(jnp.int32, s.shape, 0)
                        s = jnp.where(pos >= DIL * w, s, -1e9 * DH ** 0.5)
                    logits.append(s)
                top = functools.reduce(jnp.maximum, logits)
                e = [jnp.exp2((s - top) * (DH ** -0.5 * math.log2(math.e))) for s in logits]
                inv = 1.0 / total(e)
                for w in range(WIN):
                    probs[w, pl.ds(r, 8), :] = e[w] * inv
                if r == T - 8:
                    qkv[K, :, pl.ds(0, HALO), :] = qkv[keys, :, pl.ds(T, HALO), :]
                return probs.at[0]

            return [functools.partial(step, r=r) for r in range(0, T, 8)], WIN

        def mix_values(dst):
            def step(tie, r):
                mixed = []
                for a in range(PA):
                    o = [[] for _ in range(NT)]
                    for q in (a * rows + r, a * rows + r + 8):
                        p = [tie(probs[w, pl.ds(q, 8), :]) for w in range(WIN)]
                        for j in range(NT):
                            o[j].append(total([p[w] * qkv[V, j, pl.ds(HALO + q - DIL * w, 8), :] for w in range(WIN)]))
                    mixed.append(o)
                parts = [jnp.concatenate(from_head_minor([jnp.concatenate(c, axis=0) for c in o]), axis=1)
                         for o in mixed]
                written = store_left(parts, dst, r)
                if r == rows - 16:
                    qkv[V, :, pl.ds(0, HALO), :] = qkv[V, :, pl.ds(T, HALO), :]
                return written

            return [functools.partial(step, r=r) for r in range(0, rows, 16)], 2 * PA * WIN

        def project(line, m):
            for n in range(nt):
                cols = pl.ds(n * LANE, LANE)
                c = recombine(lambda p: line.dot(xn[p], jnp.concatenate([w[m, p, :, cols] for w in wqkv], axis=0)), PA)
                for a in range(PA):
                    for b in range(PA):
                        qkv[m, b * nt + n, pl.ds(HALO + a * rows, rows), :] = c[a][b]

        def project_first(line, m, half):
            slot = m if isinstance(m, int) else jnp.where(m == K, K0, m)
            for n in range(0, nt, 2):
                c = recombine(lambda p: line.dot(xn_first[p, :, pl.ds(half * KH, KH)],
                                                 wqkv[half][m, p, :, pl.ds(n * LANE, 2 * LANE)]), PA)
                for a in range(PA):
                    for b in range(PA):
                        for q, t in enumerate(tiles(c[a][b])):
                            at = (slot, b * nt + n + q, pl.ds(HALO + a * rows, rows), slice(None))
                            qkv[at] = t if half == 0 else qkv[at] + t

        def project_out(line, i, lhs):
            for n in range(nt):
                c = recombine(lambda p: line.dot(lhs[p], wo[p, :, pl.ds(n * LANE, LANE)]), PA)
                for a in range(PA):
                    at = pl.ds(aligned(i * T + a * rows, 16), rows)
                    for b in range(PA):
                        cols = pl.ds((b * nt + n) * LANE, LANE)
                        h_buf[at, cols] = x_buf[at, cols].astype(f32) + c[a][b]

        x_copy(0).start()
        wqkv_copy(K, 0).start()
        qkv[K0, :, pl.ds(0, HALO), :] = jnp.zeros((NT, HALO, LANE), f32)

        @apart
        def _():
            x_copy(0).wait()
            wqkv_copy(K, 1).start()
        alone(norm_x(0, xn_first))

        @apart
        def _():
            wqkv_copy(K, 0).wait()
            wqkv_copy(Q, 0).start()
        alone(projection_weights(K, 0, 64))

        def first_tile(m, _):
            after = jnp.minimum(m + 1, V)

            @apart
            def _():
                wqkv_copy(m, 1).wait()
                pl.when(m < V)(lambda: wqkv_copy(after, 1).start())
                pl.when(m == V)(lambda: x_copy(1).start())
            line = timeline()
            line.add(projection_weights(m, 1, 16), [span(0, whole // 2, 0.0, 0.85)])
            project_first(line, m, 0)
            line.run()

            @pl.when(m < V)
            def _():
                @apart
                def _():
                    wqkv_copy(after, 0).wait()
                    pl.when(m == K)(lambda: wqkv_copy(V, 0).start())
                line = timeline()
                line.add(projection_weights(after, 0, 16), [span(0, whole // 2, 0.0, 0.85)])
                project_first(line, m, 1)
                line.run()

        lax.fori_loop(0, 3, first_tile, None)

        @apart
        def _():
            wo_copy().start()
            x_copy(1).wait()
        line = timeline()
        line.add(norm_x(1, xn, tie_all=False), [span(0, whole // 2, 0.0, 0.9)], 40)
        project_first(line, V, 1)
        line.run()

        apart(lambda: start([x_copy(2)] + slice_copies(0)))
        line = timeline()
        for j in range(NT):
            qkv[V, j, pl.ds(0, HALO), :] = jnp.broadcast_to(qkv[V, j, pl.ds(HALO, 1), :], (HALO, LANE))
        line.add(scores(first=True), [span(0, whole, 0.02, 0.87)])
        project(line, K)
        line.run()

        @apart
        def _():
            wo_copy().wait()
            x_copy(3).start()
        line = timeline()
        line.add(mix_values(att), [span(0, whole, 0.0, 0.95)])
        line.add(weights(wo_raw, wo, range(D // PA // 16)), [span(0, whole, 0.0, 0.98)])
        project(line, Q)
        line.run()
        apart(lambda: start(slice_copies(1)))

        def tile(i, _):
            x_copy(i + 1).wait()
            wait(slice_copies(i - 1))

            @pl.when(i + 3 < TILES)
            def _():
                x_copy(i + 3).start()
                start(slice_copies(i + 1))

            @pl.when(i + 3 == TILES)
            def _():
                start(slice_copies(SLICES - 1, last=True))

            line = timeline()
            line.add(scores(first=False), [span(0, whole, 0.003, 1.08)], 239)
            line.add(norm_x(i + 1, xn), [span(whole, whole, 0.2, 0.796)], 156)
            line.add(mix_values(att), [span(2 * whole, whole, 0.0, 0.95)], 390)
            feed_forward_weights(line, i - 1, False,
                                 [span(0, whole, 0, 1, 0.05), span(whole, whole, 0, 1, 0.066),
                                  span(2 * whole, whole, 0, 1, 0.15), span(3 * whole, whole, 0, 0.95, 0.7)], 423)
            project(line, V)
            project_out(line, i - 1, att)
            project(line, K)
            project(line, Q)
            line.run()

        lax.fori_loop(1, TILES - 1, tile, None)

        wait(slice_copies(SLICES - 1, last=True))
        line = timeline()
        line.add(scores(first=False), [span(0, whole, 0.0, 0.9)], 310)
        line.add(mix_values(att_last), [span(whole, whole, 0.0, 0.844)], 265)
        feed_forward_weights(line, SLICES - 1, True,
                             [span(0, whole, 0, 1, 0.2), span(2 * whole, whole, 0, 0.9, 0.8)], 100)
        line.add(norm_h(0), [span(2 * whole, whole, -0.565, 0.891)], 98)
        project(line, V)
        project_out(line, TILES - 2, att)
        project_out(line, TILES - 1, att_last)
        line.run()

    left = pltpu.VMEM((products(PA), T // PA // 2, D // PA), u32)
    half = pltpu.VMEM((3, products(PA), KH // 2, D // PA), u32)
    pl.run_scoped(
        attention,
        pltpu.VMEM((S, D), bf16),
        pltpu.VMEM((PA, D // PA, 3 * D), bf16), pltpu.VMEM((PA, D // PA, D), bf16),
        pltpu.VMEM((PF, D // PF, F), bf16), pltpu.VMEM((PF, F // PF, D), bf16),
        half, half, pltpu.VMEM((products(PA), D // PA // 2, D // PA), u32),
        left, left, left, left,
        pltpu.VMEM((4, NT, HALO + T, LANE), f32), pltpu.VMEM((WIN, T, LANE), f32),
        pltpu.SemaphoreType.DMA((TILES,)), pltpu.SemaphoreType.DMA((7,)), pltpu.SemaphoreType.DMA((2 * SLICES,)),
    )

    def feed_forward(act, out_buf, out_sem):
        rows, n1, n2 = T // PF, F // PF // LANE, D // PF // LANE
        each = products(PF) * (rows // 8)

        def out_copy(i, piece):
            r, n, c = ((0, T, 0), (0, T // 2, D // 2), (T // 2, T // 2, D // 2))[piece]
            at = (pl.ds(aligned(i * T + r, 16), n), pl.ds(c, D // 2))
            return pltpu.make_async_copy(out_buf.at[at], out_hbm.at[at], out_sem.at[3 * i + piece])

        def tile(i, _):
            line = timeline()
            line.add(norm_h(jnp.minimum(i + 1, TILES - 1)),
                     [span(n1 * each, n2 * each, 0.05, 0.4), span(n1 * each, n2 * each, 0.52, 0.88)], 60)
            for n in range(n1):
                c = recombine(lambda p: line.dot(hn[p], w1[p, :, pl.ds(n * LANE, LANE)]), PF)

                def step(tie, r, n=n, c=c):
                    g = [[jnp.concatenate([tie(b[r:r + 8]), tie(b[r + 8:r + 16])], axis=0) for b in row] for row in c]
                    for p, o in enumerate(left_operands([[b * jnp.tanh(b) + b for b in row] for row in g])):
                        act.at[p][pl.ds(r // 2, 8), pl.ds(n * LANE, LANE)] = pack(o)
                    return act.at[0]

                silu = [functools.partial(step, r=r) for r in range(0, rows, 16)], 2 * PF * PF
                if n < n1 - 1:
                    line.add(silu, [span((n + 1) * each, each, -0.15, 0.45)])
                else:
                    alone(silu)
            for n in range(n2):
                c = recombine(lambda p: line.dot(act[p], w2[p, :, pl.ds(n * LANE, LANE)]), PF)
                for a in range(PF):
                    at = (pl.ds(aligned(i * T + a * rows, 16), rows), pl.ds(n * PF * LANE, PF * LANE))
                    out_buf[at] = (h_buf[at] + jnp.concatenate(c[a], axis=1)).astype(bf16)
                    if n == 1 and a == PF // 2 - 1:
                        out_copy(i, 1).start()
                if n == 0:
                    out_copy(i, 0).start()
            line.run()
            out_copy(i, 2).start()

        lax.fori_loop(0, TILES, tile, None)
        for i in range(TILES):
            for piece in range(3):
                out_copy(i, piece).wait()

    pl.run_scoped(
        feed_forward,
        pltpu.VMEM((products(PF), T // PF // 2, F // PF), u32),
        pltpu.VMEM((S, D), bf16), pltpu.SemaphoreType.DMA((3 * TILES,)),
    )


@jax.jit
def pallas_sequential_preLN__sliding_local_dilated__dense_activation_silu__prompt_kernel(
    A_x: jax.Array,
    A_wqkv: jax.Array,
    A_wo: jax.Array,
    B_x: jax.Array,
    B_w1: jax.Array,
    B_w2: jax.Array,
):
    del B_x
    hbm = pl.BlockSpec(memory_space=pl.ANY)
    out = pl.pallas_call(
        kernel,
        in_specs=[hbm] * 5,
        out_specs=hbm,
        out_shape=jax.ShapeDtypeStruct((S, D), bf16),
        scratch_shapes=[
            pltpu.VMEM((products(PF), D // PF // 2, F // PF), u32),
            pltpu.VMEM((products(PF), F // PF // 2, D // PF), u32),
            pltpu.VMEM((S, D), f32),
            pltpu.VMEM((products(PF), T // PF // 2, D // PF), u32),
            pltpu.SMEM((1,), jnp.int32),
        ],
        compiler_params=pltpu.CompilerParams(vmem_limit_bytes=124 * 2 ** 20),
    )(A_x.reshape(S, D), A_wqkv.reshape(PA, D // PA, 3 * D), A_wo.reshape(PA, D // PA, D),
      B_w1.reshape(PF, D // PF, F), B_w2.reshape(PF, F // PF, D))
    return out.reshape(1, S, D)
```
